```python
import os as _os
_os.environ.setdefault("JAX_PLATFORMS", "cpu")
import jax
import jax.numpy as jnp

def _softmax(x, axis=-1):
    return jax.nn.softmax(x, axis=axis)
def _gelu(x):
    return jax.nn.gelu(x, approximate=True)
def _silu(x):
    return jax.nn.silu(x)
def _sigmoid(x):
    return jax.nn.sigmoid(x)
def _layernorm(x, axis=-1, eps=1e-5):
    m = jnp.mean(x, axis=axis, keepdims=True)
    v = jnp.var(x, axis=axis, keepdims=True)
    return (x - m) / jnp.sqrt(v + eps)
def _scatter_add(tgt, idx, src, axis=0):
    return tgt.at[idx].add(src)
def _segment_sum(src, seg, n):
    return jax.ops.segment_sum(src, seg, n)
class _Rng:
    def __init__(self, key):
        self._k = key
    def _next(self):
        self._k, sub = jax.random.split(self._k)
        return sub
    def normal(self, shape):
        return jax.random.normal(self._next(), shape, dtype=jnp.bfloat16)
    def randint(self, lo, hi, shape):
        return jax.random.randint(self._next(), shape, lo, hi, dtype=jnp.int32)
    def uniform(self, shape, lo=0.0, hi=1.0):
        return jax.random.uniform(self._next(), shape, jnp.bfloat16, lo, hi)
    def permutation(self, n):
        return jax.random.permutation(self._next(), n)


kernel_name = 'concat_heads__gqa_block_cached__gqa_block_cached__decode'

def setup_inputs():
    _rng = _Rng(jax.random.key(int.from_bytes(__import__("os").urandom(4), "little")))
    _w = (lambda a: (lambda t: t.astype(jnp.bfloat16) if jnp.issubdtype(t.dtype, jnp.floating) else t)(jnp.asarray(a)))
    def _A_setup():
        B, Sq, D = 2, 1, 576
        Hq, Hkv, Sk, Dh = 32, 16, 4096, 128
        assert Hq % Hkv == 0, (Hq, Hkv)
        return {
            "x": _w((lambda *s: _rng.normal(s) * 0.8)(B, Sq, D)),
            "k_cache": _w((lambda *s: _rng.normal(s) * 0.8)(B, Hkv, Sk, Dh)),
            "v_cache": _w((lambda *s: _rng.normal(s) * 0.05)(B, Hkv, Sk, Dh)),
            "wq": _w((lambda *s: _rng.normal(s) * 0.8)(D, Hq * Dh) * (D ** -0.5)),
            "wo": _w((lambda *s: _rng.normal(s) * 0.05)(Hq * Dh, D) * ((Hq * Dh) ** -0.5)),
        }
    _A_in = _A_setup()

    def _B_setup():
        B, Sq, D = 2, 1, 576
        Hq, Hkv, Sk, Dh = 32, 16, 4096, 128
        assert Hq % Hkv == 0, (Hq, Hkv)
        return {
            "x": _w((lambda *s: _rng.normal(s) * 0.8)(B, Sq, D)),
            "k_cache": _w((lambda *s: _rng.normal(s) * 0.8)(B, Hkv, Sk, Dh)),
            "v_cache": _w((lambda *s: _rng.normal(s) * 0.05)(B, Hkv, Sk, Dh)),
            "wq": _w((lambda *s: _rng.normal(s) * 0.8)(D, Hq * Dh) * (D ** -0.5)),
            "wo": _w((lambda *s: _rng.normal(s) * 0.05)(Hq * Dh, D) * ((Hq * Dh) ** -0.5)),
        }
    _B_in = _B_setup()

    return {
        "A_x": _A_in["x"],
        "A_k_cache": _A_in["k_cache"],
        "A_v_cache": _A_in["v_cache"],
        "A_wq": _A_in["wq"],
        "A_wo": _A_in["wo"],
        "B_x": _B_in["x"],
        "B_k_cache": _B_in["k_cache"],
        "B_v_cache": _B_in["v_cache"],
        "B_wq": _B_in["wq"],
        "B_wo": _B_in["wo"],
    }

def reference(A_x, A_k_cache, A_v_cache, A_wq, A_wo, B_x, B_k_cache, B_v_cache, B_wq, B_wo):
    def _A_ref(x, k_cache, v_cache, wq, wo):
        B, Sq, D = x.shape
        Hq, Dh = 32, 128
        Hkv = k_cache.shape[1]
        rep = Hq // Hkv
        q = (lambda x, *d: x.transpose(*d))((x @ wq).reshape(B, Sq, Hq, Dh), 0, 2, 1, 3)
        k = jnp.repeat(k_cache, rep, axis=1)
        v = jnp.repeat(v_cache, rep, axis=1)
        scores = jnp.einsum("bhqd,bhkd->bhqk", q, k) * (Dh ** -0.5)
        p = _softmax(scores, axis=-1)
        o = jnp.einsum("bhqk,bhkd->bhqd", p, v)
        return (lambda x, *d: x.transpose(*d))(o, 0, 2, 1, 3).reshape(B, Sq, Hq * Dh) @ wo

    def _B_ref(x, k_cache, v_cache, wq, wo):
        B, Sq, D = x.shape
        Hq, Dh = 32, 128
        Hkv = k_cache.shape[1]
        rep = Hq // Hkv
        q = (lambda x, *d: x.transpose(*d))((x @ wq).reshape(B, Sq, Hq, Dh), 0, 2, 1, 3)
        k = jnp.repeat(k_cache, rep, axis=1)
        v = jnp.repeat(v_cache, rep, axis=1)
        scores = jnp.einsum("bhqd,bhkd->bhqk", q, k) * (Dh ** -0.5)
        p = _softmax(scores, axis=-1)
        o = jnp.einsum("bhqk,bhkd->bhqd", p, v)
        return (lambda x, *d: x.transpose(*d))(o, 0, 2, 1, 3).reshape(B, Sq, Hq * Dh) @ wo

    a = _A_ref(A_x, A_k_cache, A_v_cache, A_wq, A_wo)
    b = _B_ref(B_x, B_k_cache, B_v_cache, B_wq, B_wo)
    return jnp.concatenate([a, b], axis=-1)
```

```python
import functools

import jax
import jax.numpy as jnp
from jax import lax
import jax.experimental.pallas as pl
import jax.experimental.pallas.tpu as pltpu

_NT = (((1,), (1,)), ((), ()))
_BF16 = jnp.bfloat16
_F32 = jnp.float32
_TILE_ROWS = 8
_BLOCK_ROWS = 128


def _loop(lo, hi, f):
    lax.fori_loop(lo, hi, lambda i, c: f(i) or c, 0)


def _div(i, n):
    assert n & (n - 1) == 0
    return i >> (n.bit_length() - 1)


def _mod(i, n):
    assert n & (n - 1) == 0
    return i & (n - 1)


def _wait(buf, sem):
    pltpu.make_async_copy(buf, buf, sem).wait()


def _load(ref):
    return pltpu.bitcast(ref.bitcast(jnp.uint32)[...], _BF16)


def _kernel(xa_h, ka_h, va_h, wqa_h, woa_h, xb_h, kb_h, vb_h, wqb_h, wob_h, o_ref,
            x_v, kv_v, wq_v, wo_v, q_v, att_v, e_v, den_v, res_v, sem_x, sem_kv, sem_wq, sem_wo,
            *, group, period, sub, wq_rows, wq_cols, wo_rows, early, late, skew, pc, compute, wq, wo, dma):
    n_heads, seq, dh = ka_h.shape
    d_model, d_q = wqa_h.shape
    hkv = q_v.shape[1]
    n_steps = 2 * n_heads
    scale = dh ** -0.5
    w2 = 2 * dh

    full = period // sub
    rest = period - full * sub
    if 0 < rest < sub // 2:
        full, rest = full - 1, rest + sub
    parts = 2 * period * group // seq

    def fetch_kv(k_h, v_h, g, j):
        head0, slot = _mod(g * group, n_heads), lax.rem(g, 3)
        base, part = _div(j, parts) * period, _mod(j, parts)

        def fetch_rows(r, size):
            r = pl.multiple_of(r, _TILE_ROWS)
            for u in range(group):
                for s, src in enumerate((k_h, v_h)):
                    pltpu.make_async_copy(
                        src.at[head0 + u, pl.ds(r, size)],
                        kv_v.at[slot, u, s, pl.ds(r, size)],
                        sem_kv.at[slot]).start(priority=s)

        if not dma: return
        _loop(_div(part * full, parts), _div((part + 1) * full, parts),
              lambda p: fetch_rows(base + p * sub, sub))
        if rest:
            pl.when(part == parts - 1)(lambda: fetch_rows(base + full * sub, rest))

    def fetch_weights(srcs, dst, t, rows, c, size, sem):
        def copy(br, r0, rows):
            r = pl.multiple_of(r0 + t * rows, _TILE_ROWS)
            pltpu.make_async_copy(
                srcs[br].at[pl.ds(r, rows), pl.ds(c, size)],
                dst.at[pl.ds(pl.multiple_of(br * d_model + r, _TILE_ROWS), rows), pl.ds(c, size)],
                sem).start(priority=br)

        if not dma: return
        for r0 in range(0, d_model, _BLOCK_ROWS):
            for br in range(2):
                copy(br, r0, rows * min(_BLOCK_ROWS, d_model - r0) // _BLOCK_ROWS)

    def fetch_wq(t):
        c = 0
        for size in wq_cols:
            fetch_weights((wqa_h, wqb_h), wq_v, t, wq_rows, c, size, sem_wq.at[0])
            c += size

    chunk_rounds = _BLOCK_ROWS // wo_rows
    wo_rounds = d_q // pc * chunk_rounds

    def fetch_wo(lo, hi):
        def one_round(t):
            c = _div(t, chunk_rounds)
            fetch_weights((woa_h, wob_h), wo_v, _mod(t, chunk_rounds), wo_rows,
                          pl.multiple_of(c * pc, pc), pc, sem_wo.at[c])
        if wo: _loop(jnp.minimum(lo, wo_rounds), jnp.minimum(hi, wo_rounds), one_round)

    row = lax.broadcasted_iota(jnp.int32, (8, dh), 0)

    def project_q(br, h):
        x = x_v[br].astype(_F32)
        r = lax.broadcasted_iota(jnp.int32, (8, d_model), 0)
        x8 = jnp.where((r & 1) == 0, x[0:1], x[1:2]).astype(_BF16)
        w = wq_v[pl.ds(pl.multiple_of(br * d_model, 16), d_model), pl.ds(pl.multiple_of(h * w2, w2), w2)]
        q = jnp.dot(x8, w, preferred_element_type=_F32)
        q_v[br, h] = jnp.where(row < 2, q[:, :dh], q[:, dh:])

    def kv_ref(i, which):
        return kv_v.at[lax.rem(_div(i, group), 3), _mod(i, group), which]

    def scores(i):
        q = q_v[_div(i, n_heads), _mod(i, hkv)].astype(_BF16)
        s = lax.dot_general(q, _load(kv_ref(i, 0)), _NT, preferred_element_type=_F32) * scale
        e = jnp.exp(s - jnp.max(s, axis=-1, keepdims=True))
        e_v[...] = e
        den_v[...] = jnp.broadcast_to(jnp.sum(e, axis=-1, keepdims=True), den_v.shape)

    def mix_values(i):
        o = jnp.dot(e_v[...].astype(_BF16), _load(kv_ref(i, 1)), preferred_element_type=_F32)
        att_v[i] = o / den_v[...]

    def project_out(c):
        rows = []
        for br in range(2):
            cols = []
            for u in range(pc // w2):
                i = br * n_heads + c * (pc // w2) + u
                o = jnp.where((row & 1) == 0, att_v[i], att_v[i + hkv])
                cols += [jnp.where(row < 2, o, 0.0), jnp.where((row >= 2) & (row < 4), o, 0.0)]
            rows.append(jnp.concatenate(cols, axis=1))
        lhs = jnp.concatenate(rows, axis=0).astype(_BF16)
        w = wo_v[:, pl.ds(pl.multiple_of(c * pc, pc), pc)]
        res_v[...] += lax.dot_general(lhs, w, _NT, preferred_element_type=_F32)

    x_copies = [pltpu.make_async_copy(s, x_v.at[i], sem_x.at[i]) for i, s in enumerate((xa_h, xb_h))]
    for c in x_copies:
        c.start()
    if wq: _loop(0, _BLOCK_ROWS // wq_rows, fetch_wq)
    for c in x_copies:
        c.wait()
    res_v[...] = jnp.zeros_like(res_v)

    behind = 2 * group + skew
    assert early * behind + late * (d_q // pc) >= wo_rounds

    def step(n):
        g, j = _div(n, 2 * group), _mod(n, 2 * group)
        pl.when(n < 2 * n_heads)(lambda: fetch_kv(ka_h, va_h, g, j))
        pl.when((n >= 2 * n_heads) & (n < 2 * n_steps))(lambda: fetch_kv(kb_h, vb_h, g, j))

        t = jnp.maximum(n - 2 * n_steps, -1) * early
        fetch_wo(jnp.maximum(t, 0), t + early)

        i = (n - behind) >> 1
        odd = _mod(n - behind, 2) == 1

        @pl.when((i >= 0) & (_mod(n - behind, 2 * group) == 0))
        def _():
            slot = lax.rem(_div(i, group), 3)
            if dma: _wait(kv_v.at[slot], sem_kv.at[slot])

        if wq and dma: pl.when((i == -1) & odd)(lambda: _wait(wq_v, sem_wq.at[0]))
        if compute:
            pl.when((i >= 0) & ~odd)(lambda: scores(i))
            pl.when((i >= 0) & odd)(lambda: mix_values(i))
            nxt = i + 1
            if wq: pl.when(odd & (nxt >= 0) & (nxt < n_steps) & (_mod(nxt, n_heads) < hkv))(
                lambda: project_q(_div(nxt, n_heads), _mod(nxt, hkv)))

    _loop(0, 2 * n_steps + behind, step)

    def tail(c):
        t = early * behind + c * late
        fetch_wo(t, t + late)
        if dma: _wait(wo_v.at[:, pl.ds(0, pc)], sem_wo.at[c])
        if compute: project_out(c)

    if wo: _loop(0, d_q // pc, tail)

    res = res_v[...]
    lane = lax.broadcasted_iota(jnp.int32, (8, 2 * d_model), 1)
    res = jnp.where(lane < d_model, res[0:8], res[8:16])
    o_ref[...] = (res[0:2] + res[2:4]).astype(o_ref.dtype)


def build(group=4, period=1024, sub=80, wq_rows=16, wq_cols=(640,) * 5 + (896,), wo_rows=32, early=2, late=2,
          skew=1, pc=512, compute=True, wq=True, wo=True, dma=True, checks=False):
    def fn(A_x, A_k_cache, A_v_cache, A_wq, A_wo, B_x, B_k_cache, B_v_cache, B_wq, B_wo):
        batch, sq, d_model = A_x.shape
        _, hkv, seq, dh = A_k_cache.shape
        d_q = A_wq.shape[1]
        heads = lambda t: t.reshape(batch * hkv, seq, dh)
        out = pl.pallas_call(
            functools.partial(_kernel, group=group, period=period, sub=sub, wq_rows=wq_rows, wq_cols=wq_cols, wo_rows=wo_rows,
                              early=early, late=late, skew=skew, pc=pc, compute=compute, wq=wq, wo=wo, dma=dma),
            in_specs=[pl.BlockSpec(memory_space=pltpu.HBM)] * 10,
            out_specs=pl.BlockSpec(memory_space=pltpu.VMEM),
            out_shape=jax.ShapeDtypeStruct((batch, 2 * d_model), A_x.dtype),
            scratch_shapes=[
                pltpu.VMEM((2, batch, d_model), _BF16),
                pltpu.VMEM((3, group, 2, seq, dh), _BF16),
                pltpu.VMEM((2 * d_model, d_q), _BF16),
                pltpu.VMEM((2 * d_model, d_q), _BF16),
                pltpu.VMEM((2, hkv, 8, dh), _F32),
                pltpu.VMEM((2 * batch * hkv, 8, dh), _F32),
                pltpu.VMEM((8, seq), _F32),
                pltpu.VMEM((8, dh), _F32),
                pltpu.VMEM((16, 2 * d_model), _F32),
                pltpu.SemaphoreType.DMA((2,)),
                pltpu.SemaphoreType.DMA((3,)),
                pltpu.SemaphoreType.DMA((1,)),
                pltpu.SemaphoreType.DMA((d_q // pc,)),
            ],
            compiler_params=pltpu.CompilerParams(
                vmem_limit_bytes=100 * 2**20, disable_bounds_checks=not checks),
        )(A_x.reshape(batch, d_model), heads(A_k_cache), heads(A_v_cache), A_wq, A_wo.T,
          B_x.reshape(batch, d_model), heads(B_k_cache), heads(B_v_cache), B_wq, B_wo.T)
        return out.reshape(batch, sq, 2 * d_model)
    return jax.jit(fn)


pallas_concat_heads__gqa_block_cached__gqa_block_cached__decode_kernel = build(skew=2)
```

```python
import jax
import jax.numpy as jnp
from jax import lax
import jax.experimental.pallas as pl
import jax.experimental.pallas.tpu as pltpu

_BF16 = jnp.bfloat16
_F32 = jnp.float32
_NT = (((1,), (1,)), ((), ()))

_GROUP = 8
_KV_ROWS = 64
_SKEW = 2
_TILE_ROWS = 8
_BLOCK_ROWS = 64
_SPAN = 3
_WQ_COLS = 512
_WO_COLS = 512
_EARLY = 5
_LATE = 5
_LAST = ((3, 2), (2, 2))


def _loop(lo, hi, body):
    lax.fori_loop(lo, hi, lambda i, carry: body(i) or carry, 0)


def _div(i, n):
    assert n & (n - 1) == 0
    return i >> (n.bit_length() - 1)


def _mod(i, n):
    assert n & (n - 1) == 0
    return i & (n - 1)


def _aligned(start, size):
    return pl.ds(start if isinstance(start, int) else pl.multiple_of(start, size), size)


def _wait_filled(buf, sem):
    pltpu.make_async_copy(buf, buf, sem).wait()


def _kernel(xa_h, ka_h, va_h, wqa_h, woa_h, xb_h, kb_h, vb_h, wqb_h, wob_h, o_ref,
            x_v, kv_v, wq_v, wo_v, q_v, att_v, res_v, sem_x, sem_wq, sem_kv, sem_wo):
    n_heads, seq, dh = ka_h.shape
    n_blocks, _, d_q = wqa_h.shape
    d_model = n_blocks * _BLOCK_ROWS
    hkv = q_v.shape[1]
    scale = dh ** -0.5
    pair = 2 * dh
    half = _GROUP // 2
    steps = 2 * _GROUP
    last = 2 * n_heads // _GROUP - 1
    kv_steps = (last + 1) * steps
    kv_rounds = seq // (steps * _KV_ROWS)
    w_rounds = _BLOCK_ROWS // _TILE_ROWS
    n_chunks = d_q // _WO_COLS
    spans = range(0, n_blocks, _SPAN)

    def fetch_wq(t):
        n = d_q // _WQ_COLS
        rows = _aligned(_div(t, n) * _TILE_ROWS, _TILE_ROWS)
        cols = _aligned(_mod(t, n) * _WQ_COLS, _WQ_COLS)
        for b in spans:
            for br, src in enumerate((wqa_h, wqb_h)):
                pltpu.make_async_copy(
                    src.at[pl.ds(b, _SPAN), rows, cols],
                    wq_v.at[pl.ds(br * n_blocks + b, _SPAN), rows, cols], sem_wq).start(priority=br)

    def fetch_kv(k_h, v_h, g, j):
        split = g == last
        head0 = jnp.where(split, _div(j, _GROUP) * half, 0)
        head_skip = jnp.where(split, 0, half)
        row0 = jnp.where(split, _mod(j, _GROUP) * 2, j) * (kv_rounds * _KV_ROWS)
        row_step = jnp.where(split, 2 * _KV_ROWS, _KV_ROWS)
        sem = sem_kv.at[jnp.where(split & (j >= _GROUP), 2, _mod(g, 2))]
        src0 = _mod(g * _GROUP, n_heads)

        def one_round(t):
            for u in range(0, _GROUP, 2):
                h = head0 + u % half + u // half * head_skip
                rows = _aligned(row0 + t * row_step + u // half * (row_step - _KV_ROWS), _KV_ROWS)
                for s, d, n in ((0, 0, 2), (1, 0, 1), (1, 1, 1)):
                    pltpu.make_async_copy(
                        (k_h, v_h)[s].at[pl.ds(src0 + h + d, n), rows],
                        kv_v.at[_mod(g, 2), s, pl.ds(h + d, n), rows], sem).start(priority=s)

        _loop(0, kv_rounds, one_round)

    def copy_wo(br, b, n, r, c, sem):
        rows, cols = _aligned(r, _TILE_ROWS), _aligned(c * _WO_COLS, _WO_COLS)
        pltpu.make_async_copy(
            (woa_h, wob_h)[br].at[pl.ds(b, n), rows, cols],
            wo_v.at[pl.ds(br * n_blocks + b, n), rows, cols], sem_wo.at[sem]).start(priority=br)

    wo_rounds = (n_chunks - 1) * w_rounds

    def fetch_wo(lo, hi):
        def one_round(t):
            c = _div(t, w_rounds)
            for b in spans:
                for br in range(2):
                    copy_wo(br, b, _SPAN, _mod(t, w_rounds) * _TILE_ROWS, c, br * n_chunks + c)

        _loop(jnp.minimum(lo, wo_rounds), jnp.minimum(hi, wo_rounds), one_round)

    row = lax.broadcasted_iota(jnp.int32, (8, dh), 0)

    def project_q(br, h):
        x = x_v[br].astype(_F32)
        r = lax.broadcasted_iota(jnp.int32, (8, d_model), 0)
        x = jnp.where((r & 1) == 0, x[0:1], x[1:2]).astype(_BF16)
        w = wq_v[pl.ds(br * n_blocks, n_blocks), :, _aligned(h * pair, pair)]
        q = jnp.dot(x, w.reshape(d_model, pair), preferred_element_type=_F32)
        q_v[br, h] = jnp.where(row < 2, q[:, :dh], q[:, dh:])

    def attend(i):
        slot, u = _mod(_div(i, _GROUP), 2), _mod(i, _GROUP)
        q = q_v[_div(i, n_heads), _mod(i, hkv)].astype(_BF16)
        s = lax.dot_general(q, kv_v[slot, 0, u], _NT, preferred_element_type=_F32) * scale
        e = jnp.exp(s - jnp.max(s, axis=-1, keepdims=True))
        o = jnp.dot(e.astype(_BF16), kv_v[slot, 1, u], preferred_element_type=_F32)
        att_v[i] = o / jnp.sum(e, axis=-1, keepdims=True)

    def attention_outputs(c):
        rows = []
        for br in range(2):
            cols = []
            for u in range(_WO_COLS // pair):
                i = br * n_heads + c * (_WO_COLS // pair) + u
                o = jnp.where((row & 1) == 0, att_v[i], att_v[i + hkv])
                cols += [jnp.where(row < 2, o, 0.0), jnp.where((row >= 2) & (row < 4), o, 0.0)]
            rows.append(jnp.concatenate(cols, axis=1))
        return jnp.concatenate(rows, axis=0).astype(_BF16)

    def project_out(c, b, end, new, sem):
        cols = _aligned(c * _WO_COLS, _WO_COLS)
        out0, width = b * _BLOCK_ROWS, (end - b) * _BLOCK_ROWS
        lhs = attention_outputs(c)
        res = res_v[:, out0:out0 + width]
        _wait_filled(wo_v.at[pl.ds(new.start, len(new)), :, cols], sem_wo.at[sem])
        w = wo_v[b:end, :, cols].reshape(width, _WO_COLS)
        res += lax.dot_general(lhs, w, _NT, preferred_element_type=_F32)
        if isinstance(c, int) and c == n_chunks - 1:
            lane = lax.broadcasted_iota(jnp.int32, (8, width), 1)
            res = jnp.where(lane < d_model - out0, res[0:8], res[8:16])
            o_ref[:, out0:out0 + width] = (res[0:2] + res[2:4]).astype(o_ref.dtype)
        else:
            res_v[:, out0:out0 + width] = res

    def project_a(c):
        project_out(c, 0, n_blocks - 1, range(n_blocks), c)

    def project_b(c):
        project_out(c, n_blocks - 1, 2 * n_blocks, range(n_blocks, 2 * n_blocks), n_chunks + c)

    x_copies = [pltpu.make_async_copy(src, x_v.at[br], sem_x.at[br])
                for br, src in enumerate((xa_h, xb_h))]
    _loop(0, w_rounds * d_q // _WQ_COLS, fetch_wq)
    for copy in x_copies:
        copy.start()
    res_v[...] = jnp.zeros_like(res_v)

    def step(n):
        g, j = _div(n, steps), _mod(n, steps)
        pl.when(n < kv_steps // 2)(lambda: fetch_kv(ka_h, va_h, g, j))
        pl.when((n >= kv_steps // 2) & (n < kv_steps))(lambda: fetch_kv(kb_h, vb_h, g, j))
        t = jnp.maximum(n - kv_steps, -1) * _EARLY
        fetch_wo(jnp.maximum(t, 0), t + _EARLY)

        g, j = _div(n - steps - _SKEW, steps), _mod(n - steps - _SKEW, steps)

        @pl.when((g == -1) & (j == _GROUP))
        def _():
            for copy in x_copies:
                copy.wait()
            _wait_filled(wq_v, sem_wq)

        @pl.when((g >= 0) & (g < last) & (j == 0))
        def _():
            _wait_filled(kv_v.at[_mod(g, 2)], sem_kv.at[_mod(g, 2)])

        @pl.when((g == last - 1) & (j == _GROUP))
        def _():
            _wait_filled(kv_v.at[last % 2, :, pl.ds(0, half)], sem_kv.at[last % 2])

        @pl.when((g == last) & (j == 0))
        def _():
            _wait_filled(kv_v.at[last % 2, :, pl.ds(half, half)], sem_kv.at[2])

        i = g * _GROUP + j
        todo = jnp.where(g == last - 1, _GROUP + half, _GROUP)
        pl.when((g >= 0) & (j < todo))(lambda: attend(i + jnp.where(g == last, half, 0)))
        pl.when((g >= -1) & (j >= _GROUP) & (_mod(i, n_heads) < hkv))(
            lambda: project_q(_div(i, n_heads), _mod(i, hkv)))

    assert _SKEW + _GROUP <= steps
    _loop(0, kv_steps + _SKEW + half, step)

    requested = _EARLY * (_SKEW + half)
    assert all(requested + _LATE * c >= w_rounds * c for c in range(n_chunks - 1))
    assert requested + _LATE * (n_chunks - 2) >= wo_rounds

    def tail(c):
        fetch_wo(requested + c * _LATE, requested + (c + 1) * _LATE)
        project_a(c)
        pl.when(c > 0)(lambda: project_b(c - 1))

    _loop(0, n_chunks - 2, tail)

    tile_rows = range(0, _BLOCK_ROWS, _TILE_ROWS)
    last_a = [(0, b, _SPAN, r, n_chunks - 1, n_chunks - 1) for r in tile_rows for b in spans]
    last_b, ranges, b0 = [], [], 0
    for k, parts in enumerate(_LAST):
        last_b += [(1, b0 + sum(parts[:p]), n, r, n_chunks - 1, 2 * n_chunks - 1 + k)
                   for r in tile_rows for p, n in enumerate(parts)]
        ranges.append(range(n_blocks + b0, n_blocks + b0 + sum(parts)))
        b0 += sum(parts)
    assert b0 == n_blocks
    for i in range(max(len(last_a), len(last_b))):
        if i == len(last_a) // 2:
            project_a(n_chunks - 2)
        if i == len(last_a) - 1:
            project_b(n_chunks - 3)
        for todo in (last_a, last_b):
            if i < len(todo):
                copy_wo(*todo[i])
    project_a(n_chunks - 1)
    project_b(n_chunks - 2)
    for k, new in enumerate(ranges):
        project_out(n_chunks - 1, new.start - (k == 0), new.stop, new, 2 * n_chunks - 1 + k)


@jax.jit
def pallas_concat_heads__gqa_block_cached__gqa_block_cached__decode_kernel(
    A_x: jax.Array,
    A_k_cache: jax.Array,
    A_v_cache: jax.Array,
    A_wq: jax.Array,
    A_wo: jax.Array,
    B_x: jax.Array,
    B_k_cache: jax.Array,
    B_v_cache: jax.Array,
    B_wq: jax.Array,
    B_wo: jax.Array,
):
    batch, sq, d_model = A_x.shape
    _, hkv, seq, dh = A_k_cache.shape
    d_q = A_wq.shape[1]
    n_blocks = d_model // _BLOCK_ROWS
    assert (batch, sq, d_q) == (2, 1, 2 * hkv * dh) and d_model == n_blocks * _BLOCK_ROWS

    def operands(x, k, v, wq, wo):
        return (x.reshape(batch, d_model),
                k.reshape(batch * hkv, seq, dh),
                v.reshape(batch * hkv, seq, dh),
                wq.reshape(n_blocks, _BLOCK_ROWS, d_q),
                wo.T.reshape(n_blocks, _BLOCK_ROWS, d_q))

    out = pl.pallas_call(
        _kernel,
        in_specs=[pl.BlockSpec(memory_space=pltpu.HBM)] * 10,
        out_specs=pl.BlockSpec(memory_space=pltpu.VMEM),
        out_shape=jax.ShapeDtypeStruct((batch, 2 * d_model), A_x.dtype),
        scratch_shapes=[
            pltpu.VMEM((2, batch, d_model), _BF16),
            pltpu.VMEM((2, 2, _GROUP, seq, dh), _BF16),
            pltpu.VMEM((2 * n_blocks, _BLOCK_ROWS, d_q), _BF16),
            pltpu.VMEM((2 * n_blocks, _BLOCK_ROWS, d_q), _BF16),
            pltpu.VMEM((2, hkv, 8, dh), _F32),
            pltpu.VMEM((2 * batch * hkv, 8, dh), _F32),
            pltpu.VMEM((16, 2 * d_model), _F32),
            pltpu.SemaphoreType.DMA((2,)),
            pltpu.SemaphoreType.DMA(()),
            pltpu.SemaphoreType.DMA((3,)),
            pltpu.SemaphoreType.DMA((2 * d_q // _WO_COLS + len(_LAST) - 1,)),
        ],
        compiler_params=pltpu.CompilerParams(
            vmem_limit_bytes=64 * 2**20,
            disable_bounds_checks=True,
            disable_semaphore_checks=True,
        ),
    )(*operands(A_x, A_k_cache, A_v_cache, A_wq, A_wo),
      *operands(B_x, B_k_cache, B_v_cache, B_wq, B_wo))
    return out.reshape(batch, sq, 2 * d_model)
```

```python
import jax
import jax.numpy as jnp
from jax import lax
import jax.experimental.pallas as pl
import jax.experimental.pallas.tpu as pltpu

_BF16 = jnp.bfloat16
_F32 = jnp.float32
_NT = (((1,), (1,)), ((), ()))

_GROUP = 8
_KV_ROWS = 64
_SKEW = 2
_TILE_ROWS = 8
_BLOCK_ROWS = 64
_SPAN = 3
_WQ_COLS = 512
_WO_COLS = 512
_EARLY = 5
_LATE = 5
_LAST = ((3, 2), (2, 2))


def _loop(lo, hi, body):
    lax.fori_loop(lo, hi, lambda i, carry: body(i) or carry, 0)


def _div(i, n):
    assert n & (n - 1) == 0
    return i >> (n.bit_length() - 1)


def _mod(i, n):
    assert n & (n - 1) == 0
    return i & (n - 1)


def _aligned(start, size):
    return pl.ds(start if isinstance(start, int) else pl.multiple_of(start, size), size)


def _wait_filled(buf, sem):
    pltpu.make_async_copy(buf, buf, sem).wait()


def _kernel(xa_h, ka_h, va_h, wqa_h, woa_h, xb_h, kb_h, vb_h, wqb_h, wob_h, o_ref,
            x_v, kv_v, wq_v, wo_v, q_v, att_v, res_v, sem_x, sem_wq, sem_kv, sem_wo):
    n_heads, seq, dh = ka_h.shape
    n_blocks, _, d_q = wqa_h.shape
    d_model = n_blocks * _BLOCK_ROWS
    hkv = q_v.shape[1]
    scale = dh ** -0.5
    pair = 2 * dh
    half = _GROUP // 2
    steps = 2 * _GROUP
    last = 2 * n_heads // _GROUP - 1
    kv_steps = (last + 1) * steps
    kv_rounds = seq // (steps * _KV_ROWS)
    w_rounds = _BLOCK_ROWS // _TILE_ROWS
    n_chunks = d_q // _WO_COLS
    spans = range(0, n_blocks, _SPAN)

    def fetch_wq(t):
        n = d_q // _WQ_COLS
        rows = _aligned(_div(t, n) * _TILE_ROWS, _TILE_ROWS)
        cols = _aligned(_mod(t, n) * _WQ_COLS, _WQ_COLS)
        for b in spans:
            for br, src in enumerate((wqa_h, wqb_h)):
                pltpu.make_async_copy(
                    src.at[pl.ds(b, _SPAN), rows, cols],
                    wq_v.at[pl.ds(br * n_blocks + b, _SPAN), rows, cols], sem_wq).start(priority=br)

    def fetch_kv(k_h, v_h, g, j):
        split = g == last
        head0 = jnp.where(split, _div(j, _GROUP) * half, 0)
        head_skip = jnp.where(split, 0, half)
        row0 = jnp.where(split, _mod(j, _GROUP) * 2, j) * (kv_rounds * _KV_ROWS)
        row_step = jnp.where(split, 2 * _KV_ROWS, _KV_ROWS)
        sem = sem_kv.at[jnp.where(split & (j >= _GROUP), 2, _mod(g, 2))]
        src0 = _mod(g * _GROUP, n_heads)

        def one_round(t):
            for u in range(0, _GROUP, 2):
                h = head0 + u % half + u // half * head_skip
                rows = _aligned(row0 + t * row_step + u // half * (row_step - _KV_ROWS), _KV_ROWS)
                for s, src in enumerate((k_h, v_h)):
                    pltpu.make_async_copy(
                        src.at[pl.ds(src0 + h, 2), rows],
                        kv_v.at[_mod(g, 2), s, pl.ds(h, 2), rows], sem).start(priority=s)

        _loop(0, kv_rounds, one_round)

    def copy_wo(br, b, n, r, c, sem):
        rows, cols = _aligned(r, _TILE_ROWS), _aligned(c * _WO_COLS, _WO_COLS)
        pltpu.make_async_copy(
            (woa_h, wob_h)[br].at[pl.ds(b, n), rows, cols],
            wo_v.at[pl.ds(br * n_blocks + b, n), rows, cols], sem_wo.at[sem]).start(priority=br)

    wo_rounds = (n_chunks - 1) * w_rounds

    def fetch_wo(lo, hi):
        def one_round(t):
            c = _div(t, w_rounds)
            for b in spans:
                for br in range(2):
                    copy_wo(br, b, _SPAN, _mod(t, w_rounds) * _TILE_ROWS, c, br * n_chunks + c)

        _loop(jnp.minimum(lo, wo_rounds), jnp.minimum(hi, wo_rounds), one_round)

    row = lax.broadcasted_iota(jnp.int32, (8, dh), 0)

    def project_q(br, h):
        x = x_v[br].astype(_F32)
        r = lax.broadcasted_iota(jnp.int32, (8, d_model), 0)
        x = jnp.where((r & 1) == 0, x[0:1], x[1:2]).astype(_BF16)
        w = wq_v[pl.ds(br * n_blocks, n_blocks), :, _aligned(h * pair, pair)]
        q = jnp.dot(x, w.reshape(d_model, pair), preferred_element_type=_F32)
        q_v[br, h] = jnp.where(row < 2, q[:, :dh], q[:, dh:])

    def attend(i):
        slot, u = _mod(_div(i, _GROUP), 2), _mod(i, _GROUP)
        q = q_v[_div(i, n_heads), _mod(i, hkv)].astype(_BF16)
        s = lax.dot_general(q, kv_v[slot, 0, u], _NT, preferred_element_type=_F32) * scale
        e = jnp.exp(s - jnp.max(s, axis=-1, keepdims=True))
        o = jnp.dot(e.astype(_BF16), kv_v[slot, 1, u], preferred_element_type=_F32)
        att_v[i] = o / jnp.sum(e, axis=-1, keepdims=True)

    def attention_outputs(c):
        rows = []
        for br in range(2):
            cols = []
            for u in range(_WO_COLS // pair):
                i = br * n_heads + c * (_WO_COLS // pair) + u
                o = jnp.where((row & 1) == 0, att_v[i], att_v[i + hkv])
                cols += [jnp.where(row < 2, o, 0.0), jnp.where((row >= 2) & (row < 4), o, 0.0)]
            rows.append(jnp.concatenate(cols, axis=1))
        return jnp.concatenate(rows, axis=0).astype(_BF16)

    def project_out(c, b, end, new, sem):
        cols = _aligned(c * _WO_COLS, _WO_COLS)
        out0, width = b * _BLOCK_ROWS, (end - b) * _BLOCK_ROWS
        lhs = attention_outputs(c)
        res = res_v[:, out0:out0 + width]
        _wait_filled(wo_v.at[pl.ds(new.start, len(new)), :, cols], sem_wo.at[sem])
        w = wo_v[b:end, :, cols].reshape(width, _WO_COLS)
        res += lax.dot_general(lhs, w, _NT, preferred_element_type=_F32)
        if isinstance(c, int) and c == n_chunks - 1:
            lane = lax.broadcasted_iota(jnp.int32, (8, width), 1)
            res = jnp.where(lane < d_model - out0, res[0:8], res[8:16])
            o_ref[:, out0:out0 + width] = (res[0:2] + res[2:4]).astype(o_ref.dtype)
        else:
            res_v[:, out0:out0 + width] = res

    def project_a(c):
        project_out(c, 0, n_blocks - 1, range(n_blocks), c)

    def project_b(c):
        project_out(c, n_blocks - 1, 2 * n_blocks, range(n_blocks, 2 * n_blocks), n_chunks + c)

    x_copies = [pltpu.make_async_copy(src, x_v.at[br], sem_x.at[br])
                for br, src in enumerate((xa_h, xb_h))]
    _loop(0, w_rounds * d_q // _WQ_COLS, fetch_wq)
    for copy in x_copies:
        copy.start()
    res_v[...] = jnp.zeros_like(res_v)

    def step(n):
        g, j = _div(n, steps), _mod(n, steps)
        pl.when(n < kv_steps // 2)(lambda: fetch_kv(ka_h, va_h, g, j))
        pl.when((n >= kv_steps // 2) & (n < kv_steps))(lambda: fetch_kv(kb_h, vb_h, g, j))
        t = jnp.maximum(n - kv_steps, -1) * _EARLY
        fetch_wo(jnp.maximum(t, 0), t + _EARLY)

        g, j = _div(n - steps - _SKEW, steps), _mod(n - steps - _SKEW, steps)

        @pl.when((g == -1) & (j == _GROUP))
        def _():
            for copy in x_copies:
                copy.wait()
            _wait_filled(wq_v, sem_wq)

        @pl.when((g >= 0) & (g < last) & (j == 0))
        def _():
            _wait_filled(kv_v.at[_mod(g, 2)], sem_kv.at[_mod(g, 2)])

        @pl.when((g == last - 1) & (j == _GROUP))
        def _():
            _wait_filled(kv_v.at[last % 2, :, pl.ds(0, half)], sem_kv.at[last % 2])

        @pl.when((g == last) & (j == 0))
        def _():
            _wait_filled(kv_v.at[last % 2, :, pl.ds(half, half)], sem_kv.at[2])

        i = g * _GROUP + j
        todo = jnp.where(g == last - 1, _GROUP + half, _GROUP)
        pl.when((g >= 0) & (j < todo))(lambda: attend(i + jnp.where(g == last, half, 0)))
        pl.when((g >= -1) & (j >= _GROUP) & (_mod(i, n_heads) < hkv))(
            lambda: project_q(_div(i, n_heads), _mod(i, hkv)))

    assert _SKEW + _GROUP <= steps
    _loop(0, kv_steps + _SKEW + half, step)

    requested = _EARLY * (_SKEW + half)
    assert all(requested + _LATE * c >= w_rounds * c for c in range(n_chunks - 1))
    assert requested + _LATE * (n_chunks - 2) >= wo_rounds

    def tail(c):
        fetch_wo(requested + c * _LATE, requested + (c + 1) * _LATE)
        project_a(c)
        pl.when(c > 0)(lambda: project_b(c - 1))

    _loop(0, n_chunks - 2, tail)

    tile_rows = range(0, _BLOCK_ROWS, _TILE_ROWS)
    last_a = [(0, b, _SPAN, r, n_chunks - 1, n_chunks - 1) for r in tile_rows for b in spans]
    last_b, ranges, b0 = [], [], 0
    for k, parts in enumerate(_LAST):
        last_b += [(1, b0 + sum(parts[:p]), n, r, n_chunks - 1, 2 * n_chunks - 1 + k)
                   for r in tile_rows for p, n in enumerate(parts)]
        ranges.append(range(n_blocks + b0, n_blocks + b0 + sum(parts)))
        b0 += sum(parts)
    assert b0 == n_blocks
    lead = len(last_b) - len(last_a) * 2 // 3
    for i, copy_a in enumerate(last_a):
        if i == len(last_a) // 3:
            project_a(n_chunks - 2)
        if i == len(last_a) * 3 // 4:
            project_b(n_chunks - 3)
        copy_wo(*copy_a)
        if i >= lead:
            copy_wo(*last_b[i - lead])
    project_a(n_chunks - 1)
    for copy_b in last_b[len(last_a) - lead:]:
        copy_wo(*copy_b)
    project_b(n_chunks - 2)
    for k, new in enumerate(ranges):
        project_out(n_chunks - 1, new.start - (k == 0), new.stop, new, 2 * n_chunks - 1 + k)


@jax.jit
def pallas_concat_heads__gqa_block_cached__gqa_block_cached__decode_kernel(
    A_x: jax.Array,
    A_k_cache: jax.Array,
    A_v_cache: jax.Array,
    A_wq: jax.Array,
    A_wo: jax.Array,
    B_x: jax.Array,
    B_k_cache: jax.Array,
    B_v_cache: jax.Array,
    B_wq: jax.Array,
    B_wo: jax.Array,
):
    batch, sq, d_model = A_x.shape
    _, hkv, seq, dh = A_k_cache.shape
    d_q = A_wq.shape[1]
    n_blocks = d_model // _BLOCK_ROWS
    assert (batch, sq, d_q) == (2, 1, 2 * hkv * dh) and d_model == n_blocks * _BLOCK_ROWS

    def operands(x, k, v, wq, wo):
        return (x.reshape(batch, d_model),
                k.reshape(batch * hkv, seq, dh),
                v.reshape(batch * hkv, seq, dh),
                wq.reshape(n_blocks, _BLOCK_ROWS, d_q),
                wo.T.reshape(n_blocks, _BLOCK_ROWS, d_q))

    out = pl.pallas_call(
        _kernel,
        in_specs=[pl.BlockSpec(memory_space=pltpu.HBM)] * 10,
        out_specs=pl.BlockSpec(memory_space=pltpu.VMEM),
        out_shape=jax.ShapeDtypeStruct((batch, 2 * d_model), A_x.dtype),
        scratch_shapes=[
            pltpu.VMEM((2, batch, d_model), _BF16),
            pltpu.VMEM((2, 2, _GROUP, seq, dh), _BF16),
            pltpu.VMEM((2 * n_blocks, _BLOCK_ROWS, d_q), _BF16),
            pltpu.VMEM((2 * n_blocks, _BLOCK_ROWS, d_q), _BF16),
            pltpu.VMEM((2, hkv, 8, dh), _F32),
            pltpu.VMEM((2 * batch * hkv, 8, dh), _F32),
            pltpu.VMEM((16, 2 * d_model), _F32),
            pltpu.SemaphoreType.DMA((2,)),
            pltpu.SemaphoreType.DMA(()),
            pltpu.SemaphoreType.DMA((3,)),
            pltpu.SemaphoreType.DMA((2 * d_q // _WO_COLS + len(_LAST) - 1,)),
        ],
        compiler_params=pltpu.CompilerParams(
            vmem_limit_bytes=64 * 2**20,
            disable_bounds_checks=True,
            disable_semaphore_checks=True,
        ),
    )(*operands(A_x, A_k_cache, A_v_cache, A_wq, A_wo),
      *operands(B_x, B_k_cache, B_v_cache, B_wq, B_wo))
    return out.reshape(batch, sq, 2 * d_model)
```

```python
import jax
import jax.numpy as jnp
from jax import lax
import jax.experimental.pallas as pl
import jax.experimental.pallas.tpu as pltpu

_BF16 = jnp.bfloat16
_F32 = jnp.float32
_NT = (((1,), (1,)), ((), ()))

_GROUP = 8
_KV_ROWS = 64
_SKEW = 2
_TILE_ROWS = 8
_BLOCK_ROWS = 64
_SPAN = 3
_WQ_COLS = 512
_WO_COLS = 512
_EARLY = 5
_LATE = 5
_LAST = ((3, 2), (2, 2))
_LAST_LEAD = 4
_LAST_PROJECT = (12, 23)


def _loop(lo, hi, body):
    lax.fori_loop(lo, hi, lambda i, carry: body(i) or carry, 0)


def _div(i, n):
    assert n & (n - 1) == 0
    return i >> (n.bit_length() - 1)


def _mod(i, n):
    assert n & (n - 1) == 0
    return i & (n - 1)


def _aligned(start, size):
    return pl.ds(start if isinstance(start, int) else pl.multiple_of(start, size), size)


def _wait_filled(buf, sem):
    pltpu.make_async_copy(buf, buf, sem).wait()


def _kernel(xa_h, ka_h, va_h, wqa_h, woa_h, xb_h, kb_h, vb_h, wqb_h, wob_h, o_ref,
            x_v, kv_v, wq_v, wo_v, q_v, att_v, res_v, sem_x, sem_wq, sem_kv, sem_wo):
    n_heads, seq, dh = ka_h.shape
    n_blocks, _, d_q = wqa_h.shape
    d_model = n_blocks * _BLOCK_ROWS
    hkv = q_v.shape[1]
    scale = dh ** -0.5
    pair = 2 * dh
    half = _GROUP // 2
    steps = 2 * _GROUP
    last = 2 * n_heads // _GROUP - 1
    kv_steps = (last + 1) * steps
    kv_rounds = seq // (steps * _KV_ROWS)
    w_rounds = _BLOCK_ROWS // _TILE_ROWS
    n_chunks = d_q // _WO_COLS
    spans = range(0, n_blocks, _SPAN)

    def fetch_wq(t):
        n = d_q // _WQ_COLS
        rows = _aligned(_div(t, n) * _TILE_ROWS, _TILE_ROWS)
        cols = _aligned(_mod(t, n) * _WQ_COLS, _WQ_COLS)
        for b in spans:
            for br, src in enumerate((wqa_h, wqb_h)):
                pltpu.make_async_copy(
                    src.at[pl.ds(b, _SPAN), rows, cols],
                    wq_v.at[pl.ds(br * n_blocks + b, _SPAN), rows, cols], sem_wq).start(priority=br)

    def fetch_kv(k_h, v_h, g, j):
        split = g == last
        head0 = jnp.where(split, _div(j, _GROUP) * half, 0)
        head_skip = jnp.where(split, 0, half)
        row0 = jnp.where(split, _mod(j, _GROUP) * 2, j) * (kv_rounds * _KV_ROWS)
        row_step = jnp.where(split, 2 * _KV_ROWS, _KV_ROWS)
        sem = sem_kv.at[jnp.where(split & (j >= _GROUP), 2, _mod(g, 2))]
        src0 = _mod(g * _GROUP, n_heads)

        def one_round(t):
            for u in range(0, _GROUP, 2):
                h = head0 + u % half + u // half * head_skip
                rows = _aligned(row0 + t * row_step + u // half * (row_step - _KV_ROWS), _KV_ROWS)
                for s, src in enumerate((k_h, v_h)):
                    pltpu.make_async_copy(
                        src.at[pl.ds(src0 + h, 2), rows],
                        kv_v.at[_mod(g, 2), s, pl.ds(h, 2), rows], sem).start(priority=s)

        _loop(0, kv_rounds, one_round)

    def copy_wo(br, b, n, r, c, sem):
        rows, cols = _aligned(r, _TILE_ROWS), _aligned(c * _WO_COLS, _WO_COLS)
        pltpu.make_async_copy(
            (woa_h, wob_h)[br].at[pl.ds(b, n), rows, cols],
            wo_v.at[pl.ds(br * n_blocks + b, n), rows, cols], sem_wo.at[sem]).start(priority=br)

    wo_rounds = (n_chunks - 1) * w_rounds

    def fetch_wo(lo, hi):
        def one_round(t):
            c = _div(t, w_rounds)
            for b in spans:
                for br in range(2):
                    copy_wo(br, b, _SPAN, _mod(t, w_rounds) * _TILE_ROWS, c, br * n_chunks + c)

        _loop(jnp.minimum(lo, wo_rounds), jnp.minimum(hi, wo_rounds), one_round)

    row = lax.broadcasted_iota(jnp.int32, (8, dh), 0)

    def project_q(br, h):
        x = x_v[br].astype(_F32)
        r = lax.broadcasted_iota(jnp.int32, (8, d_model), 0)
        x = jnp.where((r & 1) == 0, x[0:1], x[1:2]).astype(_BF16)
        w = wq_v[pl.ds(br * n_blocks, n_blocks), :, _aligned(h * pair, pair)]
        q = jnp.dot(x, w.reshape(d_model, pair), preferred_element_type=_F32)
        q_v[br, h] = jnp.where(row < 2, q[:, :dh], q[:, dh:])

    def attend(i):
        slot, u = _mod(_div(i, _GROUP), 2), _mod(i, _GROUP)
        q = q_v[_div(i, n_heads), _mod(i, hkv)].astype(_BF16)
        s = lax.dot_general(q, kv_v[slot, 0, u], _NT, preferred_element_type=_F32) * scale
        e = jnp.exp(s - jnp.max(s, axis=-1, keepdims=True))
        o = jnp.dot(e.astype(_BF16), kv_v[slot, 1, u], preferred_element_type=_F32)
        att_v[i] = o / jnp.sum(e, axis=-1, keepdims=True)

    def attention_outputs(c):
        rows = []
        for br in range(2):
            cols = []
            for u in range(_WO_COLS // pair):
                i = br * n_heads + c * (_WO_COLS // pair) + u
                o = jnp.where((row & 1) == 0, att_v[i], att_v[i + hkv])
                cols += [jnp.where(row < 2, o, 0.0), jnp.where((row >= 2) & (row < 4), o, 0.0)]
            rows.append(jnp.concatenate(cols, axis=1))
        return jnp.concatenate(rows, axis=0).astype(_BF16)

    def project_out(c, b, end, new, sem):
        cols = _aligned(c * _WO_COLS, _WO_COLS)
        out0, width = b * _BLOCK_ROWS, (end - b) * _BLOCK_ROWS
        lhs = attention_outputs(c)
        res = res_v[:, out0:out0 + width]
        _wait_filled(wo_v.at[pl.ds(new.start, len(new)), :, cols], sem_wo.at[sem])
        w = wo_v[b:end, :, cols].reshape(width, _WO_COLS)
        res += lax.dot_general(lhs, w, _NT, preferred_element_type=_F32)
        if isinstance(c, int) and c == n_chunks - 1:
            lane = lax.broadcasted_iota(jnp.int32, (8, width), 1)
            res = jnp.where(lane < d_model - out0, res[0:8], res[8:16])
            o_ref[:, out0:out0 + width] = (res[0:2] + res[2:4]).astype(o_ref.dtype)
        else:
            res_v[:, out0:out0 + width] = res

    def project_a(c):
        project_out(c, 0, n_blocks - 1, range(n_blocks), c)

    def project_b(c):
        project_out(c, n_blocks - 1, 2 * n_blocks, range(n_blocks, 2 * n_blocks), n_chunks + c)

    x_copies = [pltpu.make_async_copy(src, x_v.at[br], sem_x.at[br])
                for br, src in enumerate((xa_h, xb_h))]
    _loop(0, w_rounds * d_q // _WQ_COLS, fetch_wq)
    for copy in x_copies:
        copy.start()
    res_v[...] = jnp.zeros_like(res_v)

    def step(n):
        g, j = _div(n, steps), _mod(n, steps)
        pl.when(n < kv_steps // 2)(lambda: fetch_kv(ka_h, va_h, g, j))
        pl.when((n >= kv_steps // 2) & (n < kv_steps))(lambda: fetch_kv(kb_h, vb_h, g, j))
        t = jnp.maximum(n - kv_steps, -1) * _EARLY
        fetch_wo(jnp.maximum(t, 0), t + _EARLY)

        g, j = _div(n - steps - _SKEW, steps), _mod(n - steps - _SKEW, steps)

        @pl.when((g == -1) & (j == _GROUP))
        def _():
            for copy in x_copies:
                copy.wait()
            _wait_filled(wq_v, sem_wq)

        @pl.when((g >= 0) & (g < last) & (j == 0))
        def _():
            _wait_filled(kv_v.at[_mod(g, 2)], sem_kv.at[_mod(g, 2)])

        @pl.when((g == last - 1) & (j == _GROUP))
        def _():
            _wait_filled(kv_v.at[last % 2, :, pl.ds(0, half)], sem_kv.at[last % 2])

        @pl.when((g == last) & (j == 0))
        def _():
            _wait_filled(kv_v.at[last % 2, :, pl.ds(half, half)], sem_kv.at[2])

        i = g * _GROUP + j
        todo = jnp.where(g == last - 1, _GROUP + half, _GROUP)
        pl.when((g >= 0) & (j < todo))(lambda: attend(i + jnp.where(g == last, half, 0)))
        pl.when((g >= -1) & (j >= _GROUP) & (_mod(i, n_heads) < hkv))(
            lambda: project_q(_div(i, n_heads), _mod(i, hkv)))

    assert _SKEW + _GROUP <= steps
    _loop(0, kv_steps + _SKEW + half, step)

    requested = _EARLY * (_SKEW + half)
    assert all(requested + _LATE * c >= w_rounds * c for c in range(n_chunks - 1))
    assert requested + _LATE * (n_chunks - 2) >= wo_rounds

    def tail(c):
        fetch_wo(requested + c * _LATE, requested + (c + 1) * _LATE)
        project_a(c)
        pl.when(c > 0)(lambda: project_b(c - 1))

    _loop(0, n_chunks - 2, tail)

    tile_rows = range(0, _BLOCK_ROWS, _TILE_ROWS)
    last_a = [(0, b, _SPAN, r, n_chunks - 1, n_chunks - 1) for r in tile_rows for b in spans]
    last_b, ranges, b0 = [], [], 0
    for k, parts in enumerate(_LAST):
        last_b += [(1, b0 + sum(parts[:p]), n, r, n_chunks - 1, 2 * n_chunks - 1 + k)
                   for r in tile_rows for p, n in enumerate(parts)]
        ranges.append(range(n_blocks + b0, n_blocks + b0 + sum(parts)))
        b0 += sum(parts)
    assert b0 == n_blocks
    for i in range(max(len(last_a), len(last_b))):
        if i == _LAST_PROJECT[0]:
            project_a(n_chunks - 2)
        if i == _LAST_PROJECT[1]:
            project_b(n_chunks - 3)
        if i < len(last_a):
            copy_wo(*last_a[i])
        if _LAST_LEAD <= i < len(last_b):
            copy_wo(*last_b[i - _LAST_LEAD])
    project_a(n_chunks - 1)
    for copy in last_b[len(last_b) - _LAST_LEAD:]:
        copy_wo(*copy)
    project_b(n_chunks - 2)
    for k, new in enumerate(ranges):
        project_out(n_chunks - 1, new.start - (k == 0), new.stop, new, 2 * n_chunks - 1 + k)


@jax.jit
def pallas_concat_heads__gqa_block_cached__gqa_block_cached__decode_kernel(
    A_x: jax.Array,
    A_k_cache: jax.Array,
    A_v_cache: jax.Array,
    A_wq: jax.Array,
    A_wo: jax.Array,
    B_x: jax.Array,
    B_k_cache: jax.Array,
    B_v_cache: jax.Array,
    B_wq: jax.Array,
    B_wo: jax.Array,
):
    batch, sq, d_model = A_x.shape
    _, hkv, seq, dh = A_k_cache.shape
    d_q = A_wq.shape[1]
    n_blocks = d_model // _BLOCK_ROWS
    assert (batch, sq, d_q) == (2, 1, 2 * hkv * dh) and d_model == n_blocks * _BLOCK_ROWS

    def operands(x, k, v, wq, wo):
        return (x.reshape(batch, d_model),
                k.reshape(batch * hkv, seq, dh),
                v.reshape(batch * hkv, seq, dh),
                wq.reshape(n_blocks, _BLOCK_ROWS, d_q),
                wo.T.reshape(n_blocks, _BLOCK_ROWS, d_q))

    out = pl.pallas_call(
        _kernel,
        in_specs=[pl.BlockSpec(memory_space=pltpu.HBM)] * 10,
        out_specs=pl.BlockSpec(memory_space=pltpu.VMEM),
        out_shape=jax.ShapeDtypeStruct((batch, 2 * d_model), A_x.dtype),
        scratch_shapes=[
            pltpu.VMEM((2, batch, d_model), _BF16),
            pltpu.VMEM((2, 2, _GROUP, seq, dh), _BF16),
            pltpu.VMEM((2 * n_blocks, _BLOCK_ROWS, d_q), _BF16),
            pltpu.VMEM((2 * n_blocks, _BLOCK_ROWS, d_q), _BF16),
            pltpu.VMEM((2, hkv, 8, dh), _F32),
            pltpu.VMEM((2 * batch * hkv, 8, dh), _F32),
            pltpu.VMEM((16, 2 * d_model), _F32),
            pltpu.SemaphoreType.DMA((2,)),
            pltpu.SemaphoreType.DMA(()),
            pltpu.SemaphoreType.DMA((3,)),
            pltpu.SemaphoreType.DMA((2 * d_q // _WO_COLS + len(_LAST) - 1,)),
        ],
        compiler_params=pltpu.CompilerParams(
            vmem_limit_bytes=64 * 2**20,
            disable_bounds_checks=True,
            disable_semaphore_checks=True,
        ),
    )(*operands(A_x, A_k_cache, A_v_cache, A_wq, A_wo),
      *operands(B_x, B_k_cache, B_v_cache, B_wq, B_wo))
    return out.reshape(batch, sq, 2 * d_model)
```
